```python
import os as _os
_os.environ.setdefault("JAX_PLATFORMS", "cpu")
import jax
import jax.numpy as jnp

def _softmax(x, axis=-1):
    return jax.nn.softmax(x, axis=axis)
def _gelu(x):
    return jax.nn.gelu(x, approximate=True)
def _silu(x):
    return jax.nn.silu(x)
def _sigmoid(x):
    return jax.nn.sigmoid(x)
def _layernorm(x, axis=-1, eps=1e-5):
    m = jnp.mean(x, axis=axis, keepdims=True)
    v = jnp.var(x, axis=axis, keepdims=True)
    return (x - m) / jnp.sqrt(v + eps)
def _scatter_add(tgt, idx, src, axis=0):
    return tgt.at[idx].add(src)
def _segment_sum(src, seg, n):
    return jax.ops.segment_sum(src, seg, n)
class _Rng:
    def __init__(self, key):
        self._k = key
    def _next(self):
        self._k, sub = jax.random.split(self._k)
        return sub
    def normal(self, shape):
        return jax.random.normal(self._next(), shape, dtype=jnp.bfloat16)
    def randint(self, lo, hi, shape):
        return jax.random.randint(self._next(), shape, lo, hi, dtype=jnp.int32)
    def uniform(self, shape, lo=0.0, hi=1.0):
        return jax.random.uniform(self._next(), shape, jnp.bfloat16, lo, hi)
    def permutation(self, n):
        return jax.random.permutation(self._next(), n)


kernel_name = 'sequential_preLN__sliding_block__swiglu_ffn__prompt'

def setup_inputs():
    _rng = _Rng(jax.random.key(int.from_bytes(__import__("os").urandom(4), "little")))
    _w = (lambda a: (lambda t: t.astype(jnp.bfloat16) if jnp.issubdtype(t.dtype, jnp.floating) else t)(jnp.asarray(a)))
    def _A_setup():
        B, S, D = 1, 2048, 512
        return {
            "x": _w((lambda *s: _rng.normal(s) * 0.05)(B, S, D)),
            "wqkv": _w((lambda *s: _rng.normal(s) * 0.05)(D, 3 * D)),
            "wo": _w((lambda *s: _rng.normal(s) * 0.05)(D, D)),
        }
    _A_in = _A_setup()

    def _B_setup():
        B, S, D, F = 1, 2048, 512, 1792
        return {
            "x": _w((lambda *s: _rng.normal(s) * 0.05)(B, S, D)),
            "w_gate": _w((lambda *s: _rng.normal(s) * 0.05)(D, F)),
            "w_up": _w((lambda *s: _rng.normal(s) * 0.05)(D, F)),
            "w_down": _w((lambda *s: _rng.normal(s) * 0.05)(F, D)),
        }
    _B_in = _B_setup()

    return {
        "A_x": _A_in["x"],
        "A_wqkv": _A_in["wqkv"],
        "A_wo": _A_in["wo"],
        "B_x": _B_in["x"],
        "B_w_gate": _B_in["w_gate"],
        "B_w_up": _B_in["w_up"],
        "B_w_down": _B_in["w_down"],
    }

def reference(A_x, A_wqkv, A_wo, B_x, B_w_gate, B_w_up, B_w_down):
    def _A_ref(x, wqkv, wo):
        B, S, D = x.shape
        H = 32; Dh = D // H; W = 256
        qkv = (lambda x, *d: x.transpose(*d))((x @ wqkv).reshape(B, S, 3, H, Dh), 2, 0, 3, 1, 4)
        q, k, v = qkv[0], qkv[1], qkv[2]
        scores = jnp.einsum("bhqd,bhkd->bhqk", q, k) * (Dh ** -0.5)
        idx = jnp.arange(S)
        mask = (idx[:, None] - idx[None, :] >= 0) & (idx[:, None] - idx[None, :] < W)
        scores = jnp.where(mask[None, None], scores, -1e9)
        p = _softmax(scores, axis=-1)
        o = jnp.einsum("bhqk,bhkd->bhqd", p, v)
        return (lambda x, *d: x.transpose(*d))(o, 0, 2, 1, 3).reshape(B, S, D) @ wo

    def _B_ref(x, w_gate, w_up, w_down):
        g = _silu(x @ w_gate)
        u = x @ w_up
        return (g * u) @ w_down

    x = A_x
    h = x + _A_ref(_layernorm(x, axis=-1), A_wqkv, A_wo)
    h2 = h + _B_ref(_layernorm(h, axis=-1), B_w_gate, B_w_up, B_w_down)
    return h2
```

```python
import functools
import math

import jax
import jax.numpy as jnp
from jax import lax
from jax.experimental import pallas as pl
from jax.experimental.pallas import tpu as pltpu

S, D, F = 2048, 512, 1792
H, DH, W = 32, 16, 256
EPS = 1e-5
F32, BF16, U32 = jnp.float32, jnp.bfloat16, jnp.uint32
NT_DIMS = (((1,), (1,)), ((), ()))


def _layernorm(x):
    m = jnp.mean(x, axis=-1, keepdims=True)
    c = x - m
    v = jnp.mean(c * c, axis=-1, keepdims=True)
    return c * lax.rsqrt(v + EPS)


def pk(x):
    return pltpu.bitcast(x.astype(BF16), U32)


def unpk(x):
    return pltpu.bitcast(x, BF16)


def pki(x):
    n, m = x.shape
    x = x.reshape(n // 16, 2, 8, m)
    lo, hi = x[:, 0].reshape(n // 2, m), x[:, 1].reshape(n // 2, m)
    return pltpu.bitcast(pltpu.pack_elementwise([lo, hi], packed_dtype=BF16), U32)


def _lhs_terms(a11, a12, a21, a22):
    return [a11 + a22, a21 + a22, a11, a22, a11 + a12, a21 - a11, a12 - a22]


_RHS = ((0, 3, 1), (0, None, 0), (1, 3, -1), (2, 0, -1), (3, None, 0), (0, 1, 1), (2, 3, 1))


def rhs_term(pi, blocks, scale=None):
    first, second, sign = _RHS[pi]
    words = [pltpu.bitcast(blocks[b], U32) for b in (first, second) if b is not None]
    if second is None and scale is None:
        return words[0]
    halves = []
    for k in range(2):
        v = [pltpu.unpack_elementwise(w, index=k, packed_dtype=BF16, unpacked_dtype=F32) for w in words]
        t = v[0] if second is None else (v[0] + v[1] if sign > 0 else v[0] - v[1])
        halves.append(t if scale is None else t * scale)
    return pltpu.bitcast(pltpu.pack_elementwise(halves, packed_dtype=BF16), U32)


def _combine(m):
    return [((m[0] + m[6]) + m[3]) - m[4], m[4] + m[2], m[3] + m[1], ((m[0] - m[1]) + m[2]) + m[5]]


ORDER = (0, 6, 3, 1, 4, 2, 5)


def _merge(*lists):
    items = []
    for li, l in enumerate(lists):
        n = len(l)
        for i, t in enumerate(l):
            items.append(((i + 0.5) / n, li, i, t))
    items.sort(key=lambda z: z[:3])
    return [t for *_, t in items]


def make_kernel(cfg):
    TM = cfg.get("TM", 256)
    G = cfg.get("G", 4)
    GPV = cfg.get("GPV", 1)
    FC = cfg.get("FC", 128)
    QS = 128 // G
    NB = S // TM
    HM, NF = TM // 2, F // 256
    NQB = TM // 128
    TOP = G // 2 if GPV == 2 else 0
    XBITS = [1 << b for b in range(int(math.log2(G))) if (1 << b) != TOP]
    ALLBITS = [1 << b for b in range(int(math.log2(G)))]
    qscale = (DH ** -0.5) * math.log2(math.e)

    def kernel(x_hbm, wqkv_hbm, wo_hbm, wg_hbm, wu_hbm, wd_hbm, out_hbm,
               x_v, wqkv_v, wo_v, wg_v, wu_v, wd_v, out_v,
               q_s, k_s, vt_s, o_s, h_s, rgu_s, rd_s,
               x_sem, w_sem, o_sem):
        def x_copy(i):
            return pltpu.make_async_copy(x_hbm.at[pl.ds(i * TM, TM)], x_v.at[pl.ds(i * TM, TM)], x_sem.at[i])

        def o_copy(i):
            r = pl.ds(i * TM, TM) if isinstance(i, int) else pl.ds(pl.multiple_of(i * TM, TM), TM)
            return pltpu.make_async_copy(out_v.at[r], out_hbm.at[r], o_sem.at[i])

        AC = cfg.get("AC", 256)
        qkv_cols = [base + c for c in range(0, D, AC) for base in (D, 0, 2 * D)]
        qkv_copies = [
            pltpu.make_async_copy(wqkv_hbm.at[:, pl.ds(c, AC)], wqkv_v.at[:, pl.ds(c, AC)], w_sem.at[4 + n])
            for n, c in enumerate(qkv_cols)]
        wo_copy = pltpu.make_async_copy(wo_hbm, wo_v, w_sem.at[0])
        wg_copy = pltpu.make_async_copy(wg_hbm, wg_v, w_sem.at[1])
        wu_copy = pltpu.make_async_copy(wu_hbm, wu_v, w_sem.at[2])
        wd_copy = pltpu.make_async_copy(wd_hbm, wd_v, w_sem.at[3])

        def rows(i, off, n):
            if isinstance(i, int):
                return pl.ds(i * TM + off, n)
            return pl.ds(pl.multiple_of(i * TM + off, 16), n)

        def prow(i, off, n):
            if isinstance(i, int):
                return pl.ds((i * TM + off) // 2, n // 2)
            return pl.ds(pl.multiple_of(i * (TM // 2) + off // 2, 8), n // 2)

        def stage_a(i):
            st = {}

            def t_ln():
                xn = _layernorm(x_v[rows(i, 0, TM), :].astype(F32))
                st["xn"] = xn.astype(BF16)
                st["xp"] = unpk(pki(xn))

            def mk(kind, c):
                def t():
                    cols = slice(c, c + AC)
                    c0 = c + {"q": 0, "k": D, "v": 2 * D}[kind]
                    r = jnp.dot(st["xp" if kind == "v" else "xn"], wqkv_v[:, c0:c0 + AC], preferred_element_type=F32)
                    if kind == "k":
                        k_s[prow(i, 0, TM), cols] = pk(r)
                    elif kind == "q":
                        q_s[prow(i, 0, TM), cols] = pk(r * qscale)
                    else:
                        for b in range(NQB):
                            vt_s[i * NQB + b, c // 2:(c + AC) // 2, :] = pk(r[b * 128:(b + 1) * 128, :].T)
                return t

            return [t_ln] + [mk(kind, c) for c in range(0, D, AC) for kind in "kqv"]

        def stage_b(i):
            first = isinstance(i, int) and i == 0
            lane8 = lax.broadcasted_iota(jnp.int32, (8, 128), 1)
            lane16 = lax.broadcasted_iota(jnp.int32, (16, 128), 1)
            lane_q = lax.broadcasted_iota(jnp.int32, (QS, 128), 1)
            row_q = lax.broadcasted_iota(jnp.int32, (QS, 128), 0)
            tri = (lane_q % QS) >= row_q
            lane_h = lax.broadcasted_iota(jnp.int32, (QS // 2, 128), 1) % QS
            sub_h = lax.broadcasted_iota(jnp.int32, (QS // 2, 128), 0)
            row_h = 16 * (sub_h // 8) + sub_h % 8
            tri_bits = (jnp.where(lane_h >= row_h, jnp.uint32(0xFFFF), jnp.uint32(0))
                        | jnp.where(lane_h >= row_h + 8, jnp.uint32(0xFFFF0000), jnp.uint32(0)))
            head_of_lane = lax.broadcasted_iota(jnp.int32, (QS // 2, 128), 1) // DH
            lane1 = lax.broadcasted_iota(jnp.int32, (1, 128), 1)

            def slot_bit0(l, b):
                return ((l // QS) & b) == 0

            groups = []
            order = [(qb, lg) for lg in range(D // 128) for qb in range(NQB)]
            for qb, lg in order:
                ot = [None] * 8
                for hg in range(8 // G):
                    st = {}
                    skip = max(0, 256 - (i * TM + qb * 128)) if first else 0

                    def t_qk(js, qb=qb, lg=lg, hg=hg, st=st, skip=skip):
                        lanes = slice(lg * 128, (lg + 1) * 128)
                        for j in js:
                            q = q_s[prow(i, qb * 128 + j * QS, QS), lanes]
                            qbd = jnp.concatenate(
                                [jnp.where(head_of_lane == hg * G + (s ^ j), q, jnp.uint32(0)) for s in range(G)], axis=0)
                            lo = max(j * QS, skip)
                            hi = j * QS + 256 + QS
                            kw = k_s[prow(i, qb * 128 - 256 + lo, hi - lo), lanes]
                            st["s", j] = lax.dot_general(unpk(kw), unpk(qbd), NT_DIMS, preferred_element_type=F32)

                    def t_sm(j, st=st, skip=skip):
                        s_t = st["s", j]
                        lo = max(j * QS, skip)
                        hi = j * QS + 256 + QS
                        last = s_t[hi - lo - QS:]
                        merged = lo == j * QS
                        if merged:
                            sm = jnp.concatenate([jnp.where(tri, last, s_t[:QS]), s_t[QS:256]], axis=0)
                        else:
                            last = jnp.where(tri, last, -jnp.inf)
                            sm = last if hi - lo == QS else jnp.concatenate([last, s_t[:hi - lo - QS]], axis=0)
                        m = jnp.max(sm, axis=0, keepdims=True)
                        n = sm.shape[0]
                        ch = cfg.get("CH", 256)
                        acc, pbs = None, []
                        for r in range(0, n, ch):
                            p = jnp.exp2(sm[r:r + ch] - m)
                            part = jnp.sum(p.reshape(-1, 8, 128), axis=0)
                            acc = part if acc is None else acc + part
                            pbs.append(pki(p))
                        st["l", j] = jnp.sum(acc, axis=0, keepdims=True)
                        pb = jnp.concatenate(pbs, axis=0)
                        d = {}
                        p_last = pb[:QS // 2] & tri_bits
                        for r in range(0, QS, 16):
                            d[hi - QS + r] = p_last[r // 2:r // 2 + 8]
                        if merged:
                            p_first = pb[:QS // 2] & ~tri_bits
                            for r in range(0, QS, 16):
                                d[lo + r] = p_first[r // 2:r // 2 + 8]
                        base = lo if merged else lo - QS
                        for r in range(QS, n, 16):
                            d[base + r] = pb[r // 2:r // 2 + 8]
                        st["p", j] = d

                    def t_pv(kts, js, qb=qb, lg=lg, hg=hg, st=st, skip=skip):
                        kts = [kt for kt in kts if kt >= skip // 128]
                        if not kts:
                            return
                        rs = [r for kt in kts for r in range(kt * 128, kt * 128 + 128, 16)]
                        if ("x", tuple(kts)) not in st:
                            z = jnp.zeros((8, 128), U32)
                            out = [[] for _ in range(G)]
                            for r in rs:
                                v = [st["p", j].get(r) for j in range(G)]
                                for b in XBITS:
                                    msk = slot_bit0(lane8, b)
                                    v = [None if v[j] is None and v[j ^ b] is None else jnp.where(
                                        msk, z if v[j] is None else v[j], z if v[j ^ b] is None else v[j ^ b])
                                        for j in range(G)]
                                for j in range(G):
                                    out[j].append(z if v[j] is None else v[j])
                            st["x", tuple(kts)] = [jnp.concatenate(o, axis=0) for o in out]

                        def vt(hd):
                            r0 = (lg * 128 + (hg * G + hd) * DH) // 2
                            return jnp.concatenate(
                                [vt_s[i * NQB + qb - 2 + kt, r0:r0 + DH // 2, :] for kt in kts], axis=1)

                        for j in js:
                            lhs = jnp.concatenate([vt(j & ~TOP), vt(j | TOP)], axis=0) if TOP else vt(j)
                            r = jnp.dot(unpk(lhs), unpk(st["x", tuple(kts)][j]), preferred_element_type=F32)
                            st["r", j] = r if ("r", j) not in st else st["r", j] + r

                    def t_fin(qb=qb, lg=lg, hg=hg, st=st, ot=ot):
                        ls = [st["l", j] for j in range(G)]
                        for b in ALLBITS:
                            msk = slot_bit0(lane1, b)
                            ls = [jnp.where(msk, ls[j], ls[j ^ b]) for j in range(G)]
                        res = [st["r", j] for j in range(G)]
                        for j in range(G):
                            if TOP:
                                r0 = DH if (j & TOP) else 0
                                o = jnp.where(slot_bit0(lane16, TOP), res[j][r0:r0 + DH], res[j ^ TOP][r0:r0 + DH])
                            else:
                                o = res[j]
                            rc = pl.reciprocal(ls[j], approx=True)
                            ot[hg * G + j] = o * (rc * (2.0 - ls[j] * rc))
                        if hg == 8 // G - 1:
                            t = pk(jnp.concatenate(ot, axis=0).T)
                            parts = [t[s * QS // 2:(s + 1) * QS // 2] for s in range(G)]
                            for b in ALLBITS:
                                msk = (head_of_lane & b) == 0
                                parts = [jnp.where(msk, parts[s], parts[s ^ b]) for s in range(G)]
                            o_s[pl.ds(qb * 64, 64), lg * 128:(lg + 1) * 128] = jnp.concatenate(parts, axis=0)

                    groups.append(dict(q=t_qk, s=t_sm, p=t_pv, f=t_fin))
            return groups

        def sched(groups, dense, pattern):
            toks = pattern.split()
            maxlag = max(int(t.split("@")[1]) for t in toks if t != "D")
            n = len(groups)
            seq = []
            for g in range(n + maxlag):
                for t in toks:
                    if t == "D":
                        seq.append(None)
                        continue
                    op, lag = t.split("@")
                    gg = g - int(lag)
                    if not 0 <= gg < n:
                        continue
                    f = groups[gg][op[0]]
                    if op[0] == "q":
                        seq.append(functools.partial(f, [int(c) for c in op[1:]] or range(G)))
                    elif op[0] == "s":
                        seq += [functools.partial(f, int(c)) for c in op[1:]]
                    elif op[0] == "p":
                        kts, _, js = op[1:].partition(":")
                        seq.append(functools.partial(f, [int(c) for c in kts], [int(c) for c in js] or range(G)))
                    else:
                        seq.append(f)
            nslots = sum(t is None for t in seq)
            out, k, done = [], 0, 0
            for t in seq:
                if t is None:
                    k += 1
                    upto = (k * len(dense)) // nslots
                    out += dense[done:upto]
                    done = upto
                else:
                    out.append(t)
            return out

        def stage_c(i, fresh=False):
            WC = cfg.get("WC", 128)
            st = {}

            def mk_wo(c):
                def t():
                    cols = slice(c, c + WC)
                    h_s[:, cols] = x_v[rows(i, 0, TM), cols].astype(F32) + jnp.dot(
                        unpk(o_s[...]), wo_v[:, cols], preferred_element_type=F32)
                return t

            def t_ln():
                hn = _layernorm(h_s[...])
                st["L"] = [t.astype(BF16) for t in _lhs_terms(
                    hn[:HM, :D // 2], hn[:HM, D // 2:], hn[HM:, :D // 2], hn[HM:, D // 2:])]

            def act(c):
                hg_ = c[:, :128]
                return (hg_ + hg_ * jnp.tanh(hg_)) * c[:, 128:]

            def mk_gu(n, pi):
                def t():
                    if fresh:
                        rhs = jnp.concatenate([rhs_term(pi, [
                            w_[r:r + D // 2, c:c + 128] for r in (0, D // 2) for c in (n * 128, F // 2 + n * 128)], sc)
                            for w_, sc in ((wg_v, 0.5), (wu_v, None))], axis=1)
                        rgu_s[pi, :, n * 256:(n + 1) * 256] = rhs
                    else:
                        rhs = rgu_s[pi, :, n * 256:(n + 1) * 256]
                    st[n, pi] = jnp.dot(st["L"][pi], unpk(rhs), preferred_element_type=F32)
                    if pi == ORDER[-1]:
                        quads = _combine([st[n, k] for k in range(7)])
                        st["D", n] = [t.astype(BF16) for t in _lhs_terms(*[act(c) for c in quads])]
                return t

            def mk_down(pi, ns, r0, r1):
                def t():
                    lhs = jnp.concatenate([st["D", n][pi][r0:r1] for n in ns], axis=1)
                    k0, k1 = ns[0] * 128, (ns[-1] + 1) * 128
                    if fresh and r0 == 0:
                        rhs = rhs_term(pi, [wd_v[r + k0:r + k1, c:c + D // 2] for r in (0, F // 2) for c in (0, D // 2)])
                        rd_s[pi, k0 // 2:k1 // 2, :] = rhs
                    else:
                        rhs = rd_s[pi, k0 // 2:k1 // 2, :]
                    y = jnp.dot(lhs, unpk(rhs), preferred_element_type=F32)
                    st.setdefault(("m", pi, r0, r1), []).append(y)
                return t

            def t_out():
                ms = []
                for pi in range(7):
                    parts = list(st.get(("m", pi, 0, HM), []))
                    if ("m", pi, 0, HM // 2) in st:
                        parts.append(jnp.concatenate([st["m", pi, 0, HM // 2][0], st["m", pi, HM // 2, HM][0]], axis=0))
                    ms.append(functools.reduce(lambda p, q: p + q, parts))
                for (r, c), y in zip(((0, 0), (0, D // 2), (HM, 0), (HM, D // 2)), _combine(ms)):
                    out_v[rows(i, r, HM), c:c + D // 2] = (h_s[r:r + HM, c:c + D // 2] + y).astype(BF16)

            pend = []
            dk = cfg.get("DK", [[0, 1], [2, 3], [4, 5], [6]])
            items = [(ns, pi) for ns in dk for pi in ORDER]
            if cfg.get("BYP", 1):
                items = [(ns, pi) for pi in ORDER for ns in dk if len(ns) % 2 == 0]
                items += [(ns, pi) for ns in dk if len(ns) % 2 for pi in ORDER]
            for ns, pi in items:
                if len(ns) % 2 and pi == ORDER[-1]:
                    pend += [(ns[-1], mk_down(pi, ns, 0, HM // 2)), (ns[-1], mk_down(pi, ns, HM // 2, HM))]
                else:
                    pend.append((ns[-1], mk_down(pi, ns, 0, HM)))
            ffn = []
            lag = cfg.get("LAG", 3)
            for k, (n, pi) in enumerate((n, pi) for n in range(NF) for pi in ORDER):
                ffn.append(mk_gu(n, pi))
                if not cfg.get("BYP", 1) and k % cfg.get("DPER", 2) == 0 and pend and (pend[0][0] + 1) * 7 + lag <= k + 1:
                    ffn.append(pend.pop(0)[1])
            ffn += [t for _, t in pend] + [t_out]
            return [mk_wo(c) for c in range(0, D, WC)], t_ln, ffn

        def run(tasks):
            for t in tasks:
                t()

        def xs_copy(i0, i1):
            r = pl.ds(i0 * TM, (i1 - i0) * TM)
            return pltpu.make_async_copy(x_hbm.at[r], x_v.at[r], x_sem.at[i0])

        x_parts = {0: xs_copy(0, 1), 1: xs_copy(1, 3), 3: xs_copy(3, NB)}
        x_parts[0].start()
        nq = len(qkv_copies)
        for c in qkv_copies:
            c.start()
        later = [[x_parts[1]], [x_parts[3]], [wg_copy, wu_copy], [wd_copy, wo_copy]]
        when = cfg.get("WHEN", [0, 3, nq, nq])
        sa = [stage_a(i) for i in range(NB)]
        x_parts[0].wait()
        sa[0][0]()
        for n in range(nq + 1):
            for cs, w in zip(later, when):
                if w == n:
                    for c in cs:
                        c.start()
            if n == cfg.get("LN1AT", nq - 1):
                x_parts[1].wait()
                sa[1][0]()
            if n < nq:
                qkv_copies[n].wait()
                sa[0][1 + n]()
        for i in range(1, NB - 1):
            if i + 1 in x_parts:
                x_parts[i + 1].wait()
            run([sa[i + 1][0]] + sa[i][1:])
        js = "".join(str(j) for j in range(G))
        run(sched(stage_b(0), sa[NB - 1][1:], cfg.get("PAT0", f"q@0 s{js}@0 D p012@2 f@2")))
        for c in (wo_copy, wg_copy, wu_copy, wd_copy):
            c.wait()

        def body(i, carry, fresh=False):
            b, (wo, ln2, ffn) = stage_b(i), stage_c(i - 1, fresh)
            dense = wo + [ln2] + [lambda: None] * cfg.get("LNAT", 0) + ffn
            npre = len(wo) + 1 if cfg.get("PRE", 1) else 0
            ntail = cfg.get("NTAIL", 0)
            run(dense[:npre])
            run(sched(b, dense[npre:len(dense) - ntail], cfg.get("PAT", f"q@0 s{js}@1 D p0@2 D p1@2 D p2@2 f@2 D")))
            run(dense[len(dense) - ntail:])
            o_copy(i - 1).start()
            return carry

        body(1, 0, True)
        if cfg.get("UNROLL", 0):
            for i in range(2, NB):
                body(i, 0)
        else:
            lax.fori_loop(2, NB, body, 0)
        wo, ln2, ffn = stage_c(NB - 1)
        run(wo + [ln2] + ffn)
        o_copy(NB - 1).start()
        for i in range(NB):
            o_copy(i).wait()

    def call(x, wqkv, wo, wg, wu, wd):
        return pl.pallas_call(
            kernel,
            out_shape=jax.ShapeDtypeStruct((S, D), BF16),
            in_specs=[pl.BlockSpec(memory_space=pl.ANY)] * 6,
            out_specs=pl.BlockSpec(memory_space=pl.ANY),
            scratch_shapes=[
                pltpu.VMEM((S, D), BF16), pltpu.VMEM((D, 3 * D), BF16), pltpu.VMEM((D, D), BF16),
                pltpu.VMEM((D, F), BF16), pltpu.VMEM((D, F), BF16), pltpu.VMEM((F, D), BF16),
                pltpu.VMEM((S, D), BF16),
                pltpu.VMEM((S // 2, D), U32), pltpu.VMEM((S // 2, D), U32),
                pltpu.VMEM((S // 128, D // 2, 128), U32),
                pltpu.VMEM((TM // 2, D), U32), pltpu.VMEM((TM, D), F32),
                pltpu.VMEM((7, D // 4, F), U32), pltpu.VMEM((7, F // 4, D // 2), U32),
                pltpu.SemaphoreType.DMA((NB,)), pltpu.SemaphoreType.DMA((4 + 3 * D // cfg.get('AC', 256),)), pltpu.SemaphoreType.DMA((NB,)),
            ],
            compiler_params=pltpu.CompilerParams(vmem_limit_bytes=64 * 2 ** 20, flags=cfg.get("flags")),
        )(x, wqkv, wo, wg, wu, wd)

    @jax.jit
    def fn(A_x, A_wqkv, A_wo, B_x, B_w_gate, B_w_up, B_w_down):
        del B_x
        return call(A_x.reshape(S, D), A_wqkv, A_wo, B_w_gate, B_w_up, B_w_down).reshape(A_x.shape)

    return fn


_fn = make_kernel(dict(NTAIL=6))


def pallas_sequential_preLN__sliding_block__swiglu_ffn__prompt_kernel(
        A_x, A_wqkv, A_wo, B_x, B_w_gate, B_w_up, B_w_down):
    return _fn(A_x, A_wqkv, A_wo, B_x, B_w_gate, B_w_up, B_w_down)


pallas_sequential_preLN__sliding_block__swiglu_ffn__prompt_kernel = jax.jit(
    pallas_sequential_preLN__sliding_block__swiglu_ffn__prompt_kernel)
```

```python
import functools
import math

import jax
import jax.numpy as jnp
from jax import lax
from jax.experimental import pallas as pl
from jax.experimental.pallas import tpu as pltpu

S, D, F = 2048, 512, 1792
DH, WIN, EPS = 16, 256, 1e-5
TM = 256
HM = TM // 2
NB, NQB, NF = S // TM, TM // 128, F // 256
G = 4
QS = 128 // G
AC = 256
QSCALE = DH ** -0.5 * math.log2(math.e)
F32, BF16, U32 = jnp.float32, jnp.bfloat16, jnp.uint32
NT_DIMS = (((1,), (1,)), ((), ()))

RHS_SIGNS = ((1, 0, 0, 1), (1, 0, 0, 0), (0, 1, 0, -1), (-1, 0, 1, 0), (0, 0, 0, 1), (1, 1, 0, 0), (0, 0, 1, 1))
ORDER = (0, 6, 3, 1, 4, 2, 5)


def _lhs_terms(a11, a12, a21, a22):
    return [a11 + a22, a21 + a22, a11, a22, a11 + a12, a21 - a11, a12 - a22]


def _combine(m):
    return [((m[0] + m[6]) + m[3]) - m[4], m[4] + m[2], m[3] + m[1], ((m[0] - m[1]) + m[2]) + m[5]]


def _bf16(words):
    return pltpu.bitcast(words, BF16)


def _half(words, k):
    return pltpu.unpack_elementwise(words, index=k, packed_dtype=BF16, unpacked_dtype=F32)


def _pack(lo, hi):
    return pltpu.bitcast(pltpu.pack_elementwise([lo, hi], packed_dtype=BF16), U32)


def _pack_rows(x):
    n, m = x.shape
    x = x.reshape(n // 16, 2, 8, m)
    return _pack(x[:, 0].reshape(n // 2, m), x[:, 1].reshape(n // 2, m))


def _unpack_rows(x):
    n, m = x.shape
    words = pltpu.bitcast(x, U32)
    return jnp.concatenate([_half(words, k).reshape(n // 16, 1, 8, m) for k in range(2)], axis=1).reshape(n, m)


def _rhs_term(signs, blocks, scale=None):
    terms = sorted(((sg, pltpu.bitcast(b, U32)) for sg, b in zip(signs, blocks) if sg), key=lambda z: -z[0])
    if len(terms) == 1 and scale is None:
        return terms[0][1]
    halves = []
    for k in range(2):
        t = None
        for sg, w in terms:
            v = _half(w, k)
            t = v if t is None else (t + v if sg > 0 else t - v)
        halves.append(t if scale is None else t * scale)
    return _pack(*halves)


def _layernorm(x):
    c = x - jnp.mean(x, axis=-1, keepdims=True)
    return c * lax.rsqrt(jnp.mean(c * c, axis=-1, keepdims=True) + EPS)


def _run(tasks):
    for t in tasks:
        t()


def _interleave(groups, dense):
    seq = []
    for g in range(len(groups) + 2):
        if g < len(groups):
            seq.append(groups[g][0])
        if 0 <= g - 1 < len(groups):
            seq += [functools.partial(groups[g - 1][1], j) for j in range(G)]
        for kt in range(3):
            seq.append(None)
            if g >= 2:
                seq.append(functools.partial(groups[g - 2][2], kt))
        if g >= 2:
            seq.append(groups[g - 2][3])
        seq.append(None)
    slots, k, done, out = sum(t is None for t in seq), 0, 0, []
    for t in seq:
        if t is None:
            k += 1
            upto = k * len(dense) // slots
            out += dense[done:upto]
            done = upto
        else:
            out.append(t)
    return out


def _kernel(x_hbm, wqkv_hbm, wo_hbm, wg_hbm, wu_hbm, wd_hbm, out_hbm,
            x_v, wqkv_v, wo_v, wg_v, wu_v, wd_v, out_v,
            wqkv_s, wo_s, q_s, k_s, vt_s, o_s, h_s, hn_s, rgu_s, rd_s,
            x_sem, w_sem, o_sem):
    recent = []

    def rows(i, off, n):
        if isinstance(i, int):
            return pl.ds(i * TM + off, n)
        return pl.ds(pl.multiple_of(i * TM + off, 16), n)

    def word_rows(i, off, n):
        if isinstance(i, int):
            return pl.ds((i * TM + off) // 2, n // 2)
        return pl.ds(pl.multiple_of(i * (TM // 2) + off // 2, 8), n // 2)

    def gate(lag, row):
        bits = pltpu.bitcast(recent[-lag][row:row + 8, :128], U32)
        return bits & (wqkv_s[:8, :128] ^ pltpu.bitcast(wqkv_v[:16, :128], U32))

    def project(i):
        st = {}

        def norm():
            xn = _layernorm(x_v[rows(i, 0, TM), :].astype(F32))
            st["k"] = xn.astype(BF16)
            st["q"] = st["v"] = _bf16(_pack_rows(xn))

        def step(kind, c):
            c0 = c + {"q": 0, "k": D, "v": 2 * D}[kind]
            if i == 0:
                w = wqkv_v[:, c0:c0 + AC]
                wqkv_s[:, c0:c0 + AC] = pltpu.bitcast(w, U32)
            else:
                w = _bf16(wqkv_s[:, c0:c0 + AC])
            r = jnp.dot(st[kind], w, preferred_element_type=F32)
            recent.extend(r[:, k:k + 128] for k in range(0, AC, 128))
            if kind == "k":
                k_s[word_rows(i, 0, TM), c:c + AC] = pltpu.bitcast(r.astype(BF16), U32)
            elif kind == "q":
                q_s[word_rows(i, 0, TM), c:c + AC] = _pack_rows(r * QSCALE)
            else:
                for b in range(NQB):
                    vt_s[i * NQB + b, c // 2:(c + AC) // 2, :] = _pack_rows(r[b * 128:(b + 1) * 128, :].T)

        return [norm] + [functools.partial(step, kind, c) for c in range(0, D, AC) for kind in "kqv"]

    def attend(i):
        static = isinstance(i, int)
        lag, stagger = (4, 64) if static else (4, 32)

        def iota(shape, dim):
            return lax.broadcasted_iota(jnp.int32, shape, dim)

        def query_of_lane(lane):
            c = lane % QS
            return (c & ~15) | ((c & 3) << 2) | ((c >> 2) & 3)

        def slot_bit_clear(lane, b):
            return ((lane // QS) & b) == 0

        lane8, lane_q, row_q = iota((8, 128), 1), iota((QS, 128), 1), iota((QS, 128), 0)
        tri = query_of_lane(lane_q) >= row_q
        lane_h, sub_h = query_of_lane(iota((QS // 2, 128), 1)), iota((QS // 2, 128), 0)
        row_h = 16 * (sub_h // 8) + sub_h % 8
        tri_bits = (jnp.where(lane_h >= row_h, jnp.uint32(0xFFFF), jnp.uint32(0))
                    | jnp.where(lane_h >= row_h + 8, jnp.uint32(0xFFFF0000), jnp.uint32(0)))
        head_of_lane = iota((QS // 2, 128), 1) // DH
        lane1 = iota((1, 128), 1)
        head_bits = [jnp.where(head_of_lane == h, jnp.uint32(0xFFFFFFFF), jnp.uint32(0)) for h in range(8)]

        def group(qb, lg, hg, heads):
            st = {}
            lanes = slice(lg * 128, (lg + 1) * 128)
            skip = max(0, WIN - (i * TM + qb * 128)) if static else 0

            def scores():
                for j in range(G):
                    q = q_s[word_rows(i, qb * 128 + j * QS, QS), lanes]
                    if len(recent) >= lag:
                        q = q | jnp.tile(gate(lag, 0), (QS // 16, 1))
                    qbd = jnp.concatenate([q & head_bits[hg * G + (s ^ j)] for s in range(G)], axis=0)
                    lo, hi = max(j * QS, skip), j * QS + WIN + QS
                    kw = k_s[word_rows(i, qb * 128 - WIN + lo, hi - lo), lanes]
                    st["s", j] = lax.dot_general(_bf16(kw), _bf16(qbd), NT_DIMS, preferred_element_type=F32)

            def row_max(j):
                s_t = st["s", j]
                lo, hi = max(j * QS, skip), j * QS + WIN + QS
                last, merged = s_t[hi - lo - QS:], lo == j * QS
                if merged:
                    sm = jnp.concatenate([jnp.where(tri, last, s_t[:QS]), s_t[QS:WIN]], axis=0)
                else:
                    last = jnp.where(tri, last, -jnp.inf)
                    sm = last if hi - lo == QS else jnp.concatenate([last, s_t[:hi - lo - QS]], axis=0)
                st["m", j] = (sm, jnp.max(sm, axis=0, keepdims=True), lo, hi, merged)
                st["p", j] = {}

            def probabilities(kt, j):
                sm, m, lo, hi, merged = st["m", j]
                base = lo if merged else lo - QS
                r0, r1 = max(QS, kt * 128 - base), min(sm.shape[0], (kt + 1) * 128 - base)
                first = ("l", j) not in st
                if first:
                    r0, r1 = 0, max(r1, QS)
                if r1 <= r0:
                    return
                if len(recent) >= lag:
                    zero = gate(lag, min(j * stagger, recent[-lag].shape[0] - 8))
                    m = pltpu.bitcast(pltpu.bitcast(jnp.broadcast_to(m, (8, 128)), U32) | zero, F32)
                    m = jnp.tile(m, ((r1 - r0) // 8, 1))
                p = jnp.exp2(sm[r0:r1] - m)
                part = jnp.sum(p.reshape(-1, 8, 128), axis=0)
                st["l", j] = part if first else st["l", j] + part
                pb, pieces = _pack_rows(p), st["p", j]
                if first:
                    p_last = pb[:QS // 2] & tri_bits
                    for r in range(0, QS, 16):
                        pieces[hi - QS + r] = p_last[r // 2:r // 2 + 8]
                    if merged:
                        p_first = pb[:QS // 2] & ~tri_bits
                        for r in range(0, QS, 16):
                            pieces[lo + r] = p_first[r // 2:r // 2 + 8]
                for r in range(max(r0, QS), r1, 16):
                    pieces[base + r] = pb[(r - r0) // 2:(r - r0) // 2 + 8]

            def values(kt):
                if kt < skip // 128:
                    return
                for j in range(G):
                    probabilities(kt, j)
                z = jnp.zeros((8, 128), U32)
                tiles = [[] for _ in range(G)]
                for r in range(kt * 128, kt * 128 + 128, 16):
                    v = [st["p", j].get(r) for j in range(G)]
                    for b in (1, 2):
                        msk = slot_bit_clear(lane8, b)
                        v = [None if v[j] is None and v[j ^ b] is None else jnp.where(
                            msk, z if v[j] is None else v[j], z if v[j ^ b] is None else v[j ^ b])
                            for j in range(G)]
                    for j in range(G):
                        tiles[j].append(z if v[j] is None else v[j])
                tiles = [jnp.concatenate(t, axis=0) for t in tiles]
                for j in range(G):
                    r0 = (lg * 128 + (hg * G + j) * DH) // 2
                    vt = vt_s[i * NQB + qb - 2 + kt, r0:r0 + DH // 2, :]
                    r = jnp.dot(_bf16(vt), _bf16(tiles[j]), preferred_element_type=F32)
                    r = [r[:8], r[8:]]
                    st["r", j] = r if ("r", j) not in st else [a + b for a, b in zip(st["r", j], r)]

            def finish():
                res = [jnp.concatenate(st["r", j], axis=0) for j in range(G)]
                ls = [jnp.sum(st["l", j], axis=0, keepdims=True) for j in range(G)]
                for b in (1, 2):
                    msk = slot_bit_clear(lane1, b)
                    ls = [jnp.where(msk, ls[j], ls[j ^ b]) for j in range(G)]
                for j in range(G):
                    rc = pl.reciprocal(ls[j], approx=True)
                    heads[hg * G + j] = res[j] * (rc * (2.0 - ls[j] * rc))
                if hg == 8 // G - 1:
                    t = _pack_rows(jnp.concatenate(heads, axis=0).T)
                    parts = [t[s * QS // 2:(s + 1) * QS // 2] for s in range(G)]
                    for b in (1, 2):
                        msk = (head_of_lane & b) == 0
                        parts = [jnp.where(msk, parts[s], parts[s ^ b]) for s in range(G)]
                    o_s[pl.ds(qb * 64, 64), lanes] = jnp.concatenate(parts, axis=0)

            return scores, row_max, values, finish

        groups = []
        for qb in range(NQB):
            for lg in range(D // 128):
                heads = [None] * 8
                groups += [group(qb, lg, hg, heads) for hg in range(8 // G)]
        return groups

    def mix(i):
        st = {}

        def step(c):
            cols = slice(c, c + 128)
            if isinstance(i, int) and i == 0:
                w = _pack_rows(wo_v[:, cols].astype(F32))
                wo_s[:, cols] = w
            else:
                w = wo_s[:, cols]
            st[c] = _unpack_rows(x_v[rows(i, 0, TM), cols]) + jnp.dot(
                _bf16(o_s[...]), _bf16(w), preferred_element_type=F32)
            h_s[rows(i, 0, TM), cols] = st[c]
            if c + 128 == D:
                hn_s[rows(i, 0, TM), :] = _layernorm(jnp.concatenate([st[k] for k in range(0, D, 128)], axis=1))

        return [functools.partial(step, c) for c in range(0, D, 128)]

    def ffn(i, fresh=False, down_last=False):
        st = {}

        def terms():
            st["L"] = [t.astype(BF16) for t in _lhs_terms(
                *[hn_s[rows(i, r, HM), c:c + D // 2] for r in (0, HM) for c in (0, D // 2)])]

        def gate_up(n, pi):
            cols = slice(n * 256, (n + 1) * 256)
            if fresh:
                rhs = jnp.concatenate([_rhs_term(RHS_SIGNS[pi], [
                    w[r:r + D // 2, c:c + 128] for r in (0, D // 2) for c in (n * 128, F // 2 + n * 128)], scale)
                    for w, scale in ((wg_v, 0.5), (wu_v, None))], axis=1)
                rgu_s[pi, :, cols] = rhs
            else:
                rhs = rgu_s[pi, :, cols]
            st[n, pi] = jnp.dot(st["L"][pi], _bf16(rhs), preferred_element_type=F32)
            recent.append(st[n, pi])
            if pi == ORDER[-1]:
                gq = _combine([st[n, k][:, :128] for k in range(7)])
                uq = _combine([st[n, k][:, 128:] for k in range(7)])
                st["D", n] = [t.astype(BF16) for t in _lhs_terms(
                    *[(g + g * jnp.tanh(g)) * u for g, u in zip(gq, uq)])]

        def down(pi, ns, r0=0, r1=HM):
            lhs = jnp.concatenate([st["D", n][pi][r0:r1] for n in ns], axis=1)
            k0, k1 = ns[0] * 128, (ns[-1] + 1) * 128
            if fresh and r0 == 0:
                rhs = _rhs_term(RHS_SIGNS[pi], [
                    wd_v[r + k0:r + k1, c:c + D // 2] for r in (0, F // 2) for c in (0, D // 2)])
                rd_s[pi, k0 // 2:k1 // 2, :] = rhs
            else:
                rhs = rd_s[pi, k0 // 2:k1 // 2, :]
            y = jnp.dot(lhs, _bf16(rhs), preferred_element_type=F32)
            st.setdefault(("m", pi, r0, r1), []).append(y)
            recent.append(y)

        def store():
            quads = []
            for c0 in (0, 128):
                ms = []
                for pi in range(7):
                    parts = [y[:, c0:c0 + 128] for y in st["m", pi, 0, HM]]
                    if ("m", pi, 0, HM // 2) in st:
                        parts.append(jnp.concatenate(
                            [st["m", pi, r, r + HM // 2][0][:, c0:c0 + 128] for r in (0, HM // 2)], axis=0))
                    ms.append(functools.reduce(lambda a, b: a + b, parts))
                quads.append(_combine(ms))
            for k in (2, 0, 1, 3):
                idx = (rows(i, (k // 2) * HM, HM), pl.ds((k % 2) * (D // 2), D // 2))
                y = jnp.concatenate([quads[0][k], quads[1][k]], axis=1)
                out_v[idx] = _bf16(_pack_rows(h_s[idx] + y))
                pltpu.make_async_copy(out_v.at[idx], out_hbm.at[idx], o_sem).start()

        def pair(a, b):
            return lambda: (down(*a), down(*b))

        pending = [(0, pair((ORDER[k], [0]), (ORDER[k + 1], [0]))) for k in (0, 2, 4)]
        pending.append((0, pair((ORDER[6], [0], 0, HM // 2), (ORDER[6], [0], HM // 2, HM))))
        chunks = [[1, 2], [3, 4], [5, 6]]
        full = [(ns, pi) for pi in ORDER for ns in chunks] if down_last else [(ns, pi) for ns in chunks for pi in ORDER]
        pending += [(ns[-1], functools.partial(down, pi, ns)) for ns, pi in full]
        tasks = [terms]
        for k in range(NF * 7):
            tasks.append(functools.partial(gate_up, k // 7, ORDER[k % 7]))
            if not down_last and pending and (pending[0][0] + 1) * 7 + 5 <= k + 1:
                tasks.append(pending.pop(0)[1])
        return tasks + [t for _, t in pending] + [store]

    def x_copy(i0, i1):
        r = pl.ds(i0 * TM, (i1 - i0) * TM)
        return pltpu.make_async_copy(x_hbm.at[r], x_v.at[r], x_sem.at[i0])

    p = [pltpu.make_async_copy(wqkv_hbm.at[:, pl.ds(c, AC)], wqkv_v.at[:, pl.ds(c, AC)], w_sem.at[4 + n])
         for n, c in enumerate(base + c for c in range(0, D, AC) for base in (D, 0, 2 * D))]
    wo_copy, wg_copy, wu_copy, wd_copy = [
        pltpu.make_async_copy(src, dst, w_sem.at[n])
        for n, (src, dst) in enumerate(((wo_hbm, wo_v), (wg_hbm, wg_v), (wu_hbm, wu_v), (wd_hbm, wd_v)))]
    x0, x1, x23, x47 = x_copy(0, 1), x_copy(1, 2), x_copy(2, 4), x_copy(4, NB)

    for c in (x0, p[0], x1, p[1], p[2], p[3]):
        c.start()
    a = [project(i) for i in range(NB)]
    x0.wait()
    a[0][0]()
    p[0].wait()
    a[0][1]()
    for c in (p[4], p[5], x23):
        c.start()
    x1.wait()
    p[1].wait()
    _run([a[1][0], a[0][2], a[1][1], a[1][2]])
    p[2].wait()
    p[3].wait()
    _run([a[0][3], a[1][3], a[0][4], a[1][4]])
    for c in (p[4], p[5], x23):
        c.wait()
    for c in (x47, wo_copy, wg_copy):
        c.start()
    _run([a[2][0], a[0][5], a[1][5], a[0][6], a[1][6]])
    _run(_interleave(attend(0), [a[3][0]] + a[2][1:] + a[3][1:-1]))
    x47.wait()
    wo_copy.wait()
    wu_copy.start()
    wd_copy.start()
    rest = []
    for i in range(4, NB):
        rest += ([a[i + 1][0]] if i + 1 < NB else []) + a[i][1:]
    _run([a[4][0]] + a[3][-1:] + mix(0))
    _run(_interleave(attend(1), rest[:-3]))
    _run(rest[-3:-2] + mix(1) + rest[-2:])
    for c in (wg_copy, wu_copy, wd_copy):
        c.wait()
    _run(ffn(0, fresh=True, down_last=True))

    def body(i, carry):
        del recent[:]
        dense = ffn(i - 1)
        _run(_interleave(attend(i), dense[:-7]))
        _run(dense[-7:-6] + mix(i) + dense[-6:])
        return carry

    lax.fori_loop(2, NB, body, 0)
    _run(ffn(NB - 1, down_last=True))
    pltpu.make_async_copy(out_v, out_hbm, o_sem).wait()


@jax.jit
def pallas_sequential_preLN__sliding_block__swiglu_ffn__prompt_kernel(
    A_x: jax.Array,
    A_wqkv: jax.Array,
    A_wo: jax.Array,
    B_x: jax.Array,
    B_w_gate: jax.Array,
    B_w_up: jax.Array,
    B_w_down: jax.Array,
):
    del B_x
    out = pl.pallas_call(
        _kernel,
        out_shape=jax.ShapeDtypeStruct((S, D), BF16),
        in_specs=[pl.BlockSpec(memory_space=pl.ANY)] * 6,
        out_specs=pl.BlockSpec(memory_space=pl.ANY),
        scratch_shapes=[
            pltpu.VMEM((S, D), BF16), pltpu.VMEM((D, 3 * D), BF16), pltpu.VMEM((D, D), BF16),
            pltpu.VMEM((D, F), BF16), pltpu.VMEM((D, F), BF16), pltpu.VMEM((F, D), BF16),
            pltpu.VMEM((S, D), BF16),
            pltpu.VMEM((D // 2, 3 * D), U32), pltpu.VMEM((D // 2, D), U32),
            pltpu.VMEM((S // 2, D), U32), pltpu.VMEM((S // 2, D), U32),
            pltpu.VMEM((S // 128, D // 2, 128), U32),
            pltpu.VMEM((TM // 2, D), U32), pltpu.VMEM((S, D), F32), pltpu.VMEM((S, D), F32),
            pltpu.VMEM((7, D // 4, F), U32), pltpu.VMEM((7, F // 4, D // 2), U32),
            pltpu.SemaphoreType.DMA((NB,)), pltpu.SemaphoreType.DMA((4 + 3 * D // AC,)),
            pltpu.SemaphoreType.DMA(()),
        ],
        compiler_params=pltpu.CompilerParams(vmem_limit_bytes=64 * 2 ** 20),
    )(A_x.reshape(S, D), A_wqkv, A_wo, B_w_gate, B_w_up, B_w_down)
    return out.reshape(A_x.shape)
```
